```python
import os as _os
_os.environ.setdefault("JAX_PLATFORMS", "cpu")
import jax
import jax.numpy as jnp

def _softmax(x, axis=-1):
    return jax.nn.softmax(x, axis=axis)
def _gelu(x):
    return jax.nn.gelu(x, approximate=True)
def _silu(x):
    return jax.nn.silu(x)
def _sigmoid(x):
    return jax.nn.sigmoid(x)
def _layernorm(x, axis=-1, eps=1e-5):
    m = jnp.mean(x, axis=axis, keepdims=True)
    v = jnp.var(x, axis=axis, keepdims=True)
    return (x - m) / jnp.sqrt(v + eps)
def _scatter_add(tgt, idx, src, axis=0):
    return tgt.at[idx].add(src)
def _segment_sum(src, seg, n):
    return jax.ops.segment_sum(src, seg, n)
class _Rng:
    def __init__(self, key):
        self._k = key
    def _next(self):
        self._k, sub = jax.random.split(self._k)
        return sub
    def normal(self, shape):
        return jax.random.normal(self._next(), shape, dtype=jnp.bfloat16)
    def randint(self, lo, hi, shape):
        return jax.random.randint(self._next(), shape, lo, hi, dtype=jnp.int32)
    def uniform(self, shape, lo=0.0, hi=1.0):
        return jax.random.uniform(self._next(), shape, jnp.bfloat16, lo, hi)
    def permutation(self, n):
        return jax.random.permutation(self._next(), n)


kernel_name = 'gated_mix__mha_block__mixer_s_mlp__prompt'

def setup_inputs():
    _rng = _Rng(jax.random.key(int.from_bytes(__import__("os").urandom(4), "little")))
    _w = (lambda a: (lambda t: t.astype(jnp.bfloat16) if jnp.issubdtype(t.dtype, jnp.floating) else t)(jnp.asarray(a)))
    def _A_setup():
        B, S, D, H = 1, 2048, 512, 32
        return {
            "x": _w((lambda *s: _rng.normal(s) * 0.05)(B, S, D)),
            "wqkv": _w((lambda *s: _rng.normal(s) * 0.8)(D, 3 * D)),
            "wo": _w((lambda *s: _rng.normal(s) * 0.05)(D, D)),
        }
    _A_in = _A_setup()

    def _B_setup():
        B, S, D, F = 1, 2048, 512, 1792
        return {
            "x":  _w((lambda *s: _rng.normal(s) * 0.05)(B, S, D)),
            "w1": _w((lambda *s: _rng.normal(s) * 0.2)(D, D) * (D ** -0.5)),
            "w2": _w((lambda *s: _rng.normal(s) * 0.2)(D, D) * (D ** -0.5)),
            "w3": _w((lambda *s: _rng.normal(s) * 0.2)(D, F) * (D ** -0.5)),
            "w4": _w((lambda *s: _rng.normal(s) * 0.2)(F, D) * (F ** -0.5)),
        }
    _B_in = _B_setup()

    return {
        "A_x": _A_in["x"],
        "A_wqkv": _A_in["wqkv"],
        "A_wo": _A_in["wo"],
        "B_x": _B_in["x"],
        "B_w1": _B_in["w1"],
        "B_w2": _B_in["w2"],
        "B_w3": _B_in["w3"],
        "B_w4": _B_in["w4"],
        "gate_w": _w((lambda *s: _rng.normal(s) * 0.05)(512) * 16.0),
    }

def reference(A_x, A_wqkv, A_wo, B_x, B_w1, B_w2, B_w3, B_w4, gate_w):
    def _A_ref(x, wqkv, wo):
        B, S, D = x.shape
        H = 32
        Dh = D // H
        qkv = (lambda x, *d: x.transpose(*d))((x @ wqkv).reshape(B, S, 3, H, Dh), 2, 0, 3, 1, 4)
        q, k, v = qkv[0], qkv[1], qkv[2]
        scores = jnp.einsum("bhqd,bhkd->bhqk", q, k) * (Dh ** -0.5)
        p = _softmax(scores, axis=-1)
        o = jnp.einsum("bhqk,bhkd->bhqd", p, v)
        return (lambda x, *d: x.transpose(*d))(o, 0, 2, 1, 3).reshape(B, S, D) @ wo

    def _B_ref(x, w1, w2, w3, w4):
        B, S, D = x.shape
        h = _gelu(_layernorm(x, axis=-1) @ w1)
        c = D // 4
        g0 = jnp.pad(h[:, :, 0*c:1*c], ((0, 0), (1, 0), (0, 0)))[:, :S, :]
        g1 = jnp.pad(h[:, :, 1*c:2*c], ((0, 0), (0, 1), (0, 0)))[:, 1:, :]
        g2 = jnp.pad(h[:, :, 2*c:3*c], ((0, 0), (2, 0), (0, 0)))[:, :S, :]
        g3 = jnp.pad(h[:, :, 3*c:   ], ((0, 0), (0, 2), (0, 0)))[:, 2:, :]
        hs = jnp.concatenate([g0, g1, g2, g3], axis=-1) @ w2
        x1 = x + hs
        h2 = _gelu(_layernorm(x1, axis=-1) @ w3) @ w4
        return x1 + h2

    x = A_x
    g = _sigmoid((x * gate_w).sum(-1, keepdims=True))
    a = _A_ref(x, A_wqkv, A_wo)
    b = _B_ref(x, B_w1, B_w2, B_w3, B_w4)
    return g * a + (1 - g) * b
```

```python
import functools, os
import math

import jax
import jax.numpy as jnp
import jax.experimental.pallas as pl
import jax.experimental.pallas.tpu as pltpu

S = 2048
D = 512
H = 32
DH = 16
F = 1792
HG = 8
NG = H // HG
BQ = S
KC = 128
NC = S // KC
QW = int(os.environ.get('QW', 512))
NQ = BQ // QW
PAD = 8
PRO = 256
NPRO = S // PRO
MB = 256
NMB = S // MB
EPS = 1e-5
QSCALE = (DH ** -0.5) * math.log2(math.e)
KV = int(os.environ.get('KV', 0))
KV0 = S - KV
LAG = int(os.environ.get('LAG', 1))
V_END = int(os.environ.get('V_END', 46))
FORCE = int(os.environ.get('FORCE', -1))
SCORE_BOUND = 60.0
V_MAX = 2.0 ** 50
V_MIN = 2.0 ** -24

_F32 = jnp.float32
_BF16 = jnp.bfloat16


def _dot(a, b):
    return jnp.dot(a, b, preferred_element_type=_F32)


def _dot_nt(a, b):
    return jax.lax.dot_general(a, b, (((1,), (1,)), ((), ())),
                               preferred_element_type=_F32)


def _ln(x):
    m = jnp.mean(x, axis=-1, keepdims=True)
    xc = x - m
    v = jnp.mean(xc * xc, axis=-1, keepdims=True)
    return xc / jnp.sqrt(v + EPS)


def _gelu(x):
    c = math.sqrt(2.0 / math.pi)
    return 0.5 * x * (1.0 + jnp.tanh(c * (x + 0.044715 * (x * x * x))))


def _fold8(x, op):
    return op(x.reshape(x.shape[0] // 8, 8, x.shape[1]), axis=0)


def _kernel(x_hbm, wqkv_hbm, wo_hbm, w1_hbm, w2_hbm, w3_hbm, w4_hbm,
            gw_ref, o_hbm,
            x_v, wqkv_v, wo_v, w1_v, w2_v, w3_v, w4_v, sems, osems, o_buf,
            k_sc, vt_sc, qt_sc, h_sc, ot_sc, wt_sc, sa, pa, la,
            kv_sc, kb, qb, g_sc, x1_sc, xn_sc, flag):

    def x_copy(c):
        return pltpu.make_async_copy(x_hbm.at[pl.ds(c * PRO, PRO), :],
                                     x_v.at[pl.ds(c * PRO, PRO), :],
                                     sems.at[c])

    def w_copy(i):
        src, dst = [(wqkv_hbm, wqkv_v), (w1_hbm, w1_v), (wo_hbm, wo_v),
                    (w2_hbm, w2_v), (w3_hbm, w3_v), (w4_hbm, w4_v)][i]
        return pltpu.make_async_copy(src, dst, sems.at[NPRO + i])

    def o_copy(mb, slot):
        return pltpu.make_async_copy(o_buf.at[slot],
                                     o_hbm.at[pl.ds(mb * MB, MB), :],
                                     osems.at[slot])

    w_copy(1).start()
    x_copy(0).start()
    w_copy(0).start()
    for c in range(1, NPRO):
        x_copy(c).start()
    h_sc[0:PAD, :] = jnp.zeros((PAD, D), _F32)
    h_sc[PAD + S:PAD + S + PAD, :] = jnp.zeros((PAD, D), _F32)
    g_sc[0] = jnp.zeros((H, PRO), _F32)
    g_sc[1] = jnp.zeros((H, PRO), _F32)
    w_copy(1).wait()

    grp = (jax.lax.broadcasted_iota(jnp.int32, (H, D), 1) // DH ==
           jax.lax.broadcasted_iota(jnp.int32, (H, D), 0)
           ).astype(_F32).astype(_BF16)

    def pro_part(c, vmax, do_h, do_qkv):
        if do_h:
            r1 = pl.multiple_of((c + 1) * PRO, PRO)
            x_copy(c + 1).wait()
        if do_qkv:
            r0 = pl.multiple_of(c * PRO, PRO)
            x = x_v[pl.ds(r0, PRO), :]
            k = _dot(x, wqkv_v[:, D:2 * D]).astype(_BF16)
            for g in range(NG):
                k_sc[g, pl.ds(r0, PRO), :] = k[:, g * 128:(g + 1) * 128]
        if do_h:
            xn = _ln(x_v[pl.ds(r1, PRO), :].astype(_F32)).astype(_BF16)
        if do_qkv:
            qt = (_dot_nt(wt_sc[0], x) * QSCALE).astype(_BF16)
            qt_sc[:, pl.ds(r0, PRO)] = qt
        if do_h:
            hpre = _dot(xn, w1_v[...])
        if do_qkv:
            vt = _dot_nt(wt_sc[1], x).astype(_BF16)
            vt_sc[:, pl.ds(r0, PRO)] = vt
        if do_h:
            h_sc[pl.ds(PAD + r1, PRO), :] = (
                _gelu(hpre).astype(_BF16).astype(_F32))
        if do_qkv:
            k32 = k.astype(_F32)
            q32 = qt.astype(_F32)
            g_sc[0] = jnp.maximum(g_sc[0],
                                  _dot(grp, (q32 * q32).astype(_BF16)))
            g_sc[1] = jnp.maximum(g_sc[1],
                                  _dot_nt(grp, (k32 * k32).astype(_BF16)))
            vmax = jnp.maximum(vmax,
                               _fold8(jnp.abs(vt.astype(_F32)).T, jnp.max))
        return vmax

    pro_part(-1, None, True, False)
    w_copy(0).wait()
    for i in (3, 2, 4, 5):
        w_copy(i).start()
    wt_sc[0] = wqkv_v[:, 0:D].astype(_F32).T.astype(_BF16)
    wt_sc[1] = wqkv_v[:, 2 * D:3 * D].astype(_F32).T.astype(_BF16)

    vmax = jax.lax.fori_loop(
        0, NPRO - 1, lambda c, vm: pro_part(c, vm, True, True),
        jnp.zeros((8, D), _F32))
    vmax = pro_part(NPRO - 1, vmax, False, True)
    vcol = jnp.max(vmax, axis=0, keepdims=True)
    q2 = jnp.max(g_sc[0], axis=1, keepdims=True)
    k2 = jnp.max(g_sc[1], axis=1, keepdims=True)
    ok_s = (q2 * k2 * 1.03 <= SCORE_BOUND * SCORE_BOUND).astype(_F32)
    ok_v = ((vcol <= V_MAX) & ((vcol >= V_MIN) | (vcol == 0.0))).astype(_F32)
    ok = jnp.minimum(jnp.min(ok_s), jnp.min(ok_v))
    flag[0] = (ok > 0.5).astype(jnp.int32)
    if FORCE >= 0:
        flag[0] = FORCE

    rows = jax.lax.broadcasted_iota(jnp.int32, (128, BQ), 0)

    def make_qm(h):
        g = h // HG
        hl = h % HG
        qg = qt_sc[pl.ds(pl.multiple_of(g * 128, 128), 128), :]
        return g, jnp.where((rows >> 4) == hl, qg, jnp.zeros_like(qg))

    NVC = -(-KV // KC)
    order = list(range(NC - NVC, NC)) + list(range(NC - NVC))

    def prep_pieces(h):
        h = jnp.minimum(h, H - 1)
        out = []

        def q_piece(d0):
            def run():
                q = qt_sc[pl.ds(pl.multiple_of(h * DH, DH), DH), :].astype(_F32)
                for d in range(d0, d0 + 4):
                    qb[d] = jnp.broadcast_to(q[d:d + 1, :], (8, BQ))
            return run

        def k_piece(d0):
            def run():
                k = kv_sc[h]
                for d in range(d0, d0 + 2):
                    kb[d] = jnp.broadcast_to(k[:, d:d + 1], (KV, 128))
            return run

        if KV:
            out += [k_piece(d0) for d0 in range(0, DH, 2)]
            out += [q_piece(d0) for d0 in range(0, DH, 4)]
        return out

    def vpu_piece(i, j, dep):
        r0 = i * 16
        lsum = []
        for nb in range(QW // 256):
            ns = slice(j * QW + nb * 256, j * QW + (nb + 1) * 256)
            acc = None
            for d in range(DH):
                kk = kb[d, r0:r0 + 16, :]
                qq = qb[d, :, ns]
                if d == 0 and dep is not None:
                    qq = qq + jnp.minimum(
                        dep[0:8, nb * 256:(nb + 1) * 256], 0.0)
                tt = (jnp.concatenate([kk, kk], axis=1) *
                      jnp.concatenate([qq, qq], axis=0))
                acc = tt if acc is None else acc + tt
            p = jnp.exp2(acc)
            pa[KV0 + r0:KV0 + r0 + 16, ns] = p.astype(_BF16)
            lsum.append(p[0:8] + p[8:16])
        return jnp.concatenate(lsum, axis=1)

    def fstage(h, do_pv, do_qk):
        o = [None] * NQ
        l_new = [None] * NQ
        if do_pv:
            l_old = jnp.sum(la[...], axis=0, keepdims=True)
            v_off = pl.multiple_of(h * DH, DH)
        if do_qk:
            g, qm = make_qm(h + 1)
            vp = [(((KV0 + i * 16) // KC - (NC - NVC)) * NQ + j, i, j)
                  for i in range(KV // 16) for j in range(NQ)]
            vp.sort()
            preps = prep_pieces(h + 2)
        else:
            vp, preps = [], []
        n_vp, n_pr = len(vp), len(preps)
        nslot = NC * NQ
        deps = [None] * (LAG + 1)
        slot = 0
        for pos, c in enumerate(order):
            lo, hi = c * KC, min((c + 1) * KC, KV0)
            for j in range(NQ):
                qs = slice(j * QW, (j + 1) * QW)
                if do_pv:
                    ks = slice(c * KC, (c + 1) * KC)
                    oc = _dot(vt_sc[pl.ds(v_off, DH), ks], pa[ks, qs])
                    o[j] = oc if o[j] is None else o[j] + oc
                if do_qk and hi > lo:
                    p = jnp.exp2(_dot(k_sc[g, lo:hi, :], qm[:, qs]))
                    pa[lo:hi, qs] = p.astype(_BF16)
                    lc = _fold8(p, jnp.sum)
                    l_new[j] = lc if l_new[j] is None else l_new[j] + lc
                    deps.append(p)
                else:
                    deps.append(None)
                while (vp and vp[0][0] <= slot and
                       (n_vp - len(vp)) * (V_END + 1) < (slot + 1) * n_vp):
                    _, i, jj = vp.pop(0)
                    lc = vpu_piece(i, jj, deps[-1 - LAG])
                    l_new[jj] = lc if l_new[jj] is None else l_new[jj] + lc
                if not vp and preps and slot > V_END:
                    left = nslot - slot
                    for _ in range(-(-len(preps) // left)):
                        preps.pop(0)()
                slot += 1
        assert not vp and not preps
        if do_pv:
            ot_sc[pl.ds(v_off, DH), :] = jnp.concatenate(o, axis=1) / l_old
        if do_qk:
            la[...] = jnp.concatenate(l_new, axis=1)

    @pl.when(flag[0] == 1)
    def _prep0():
        for g in range(NG if KV else 0):
            kg = k_sc[g, KV0:S, :].astype(_F32)
            for hl in range(HG):
                kv_sc[g * HG + hl] = (
                    kg if hl == 0 else pltpu.roll(kg, 128 - hl * DH, 1))

    @pl.when(flag[0] == 1)
    def _prep1():
        for run in prep_pieces(0):
            run()

    @pl.when(flag[0] == 1)
    def _fast():
        fstage(-1, False, True)

        def body(h, carry):
            fstage(h, True, True)
            return carry

        jax.lax.fori_loop(0, H - 1, body, 0)
        fstage(H - 1, True, False)

    @pl.when(flag[0] != 1)
    def _general():
        def head(h, carry):
            g, qm = make_qm(h)
            v_off = pl.multiple_of(h * DH, DH)

            def pass1(c, m):
                ks = pl.ds(pl.multiple_of(c * KC, KC), KC)
                s = _dot(k_sc[g, ks, :], qm)
                sa[ks, :] = s
                return jnp.maximum(m, _fold8(s, jnp.max))

            m8 = jax.lax.fori_loop(
                0, NC, pass1, jnp.full((8, BQ), -jnp.inf, _F32))
            m = jnp.max(m8, axis=0, keepdims=True)

            def pass2(c, carry2):
                o, l = carry2
                ks = pl.ds(pl.multiple_of(c * KC, KC), KC)
                p = jnp.exp2(sa[ks, :] - m)
                o = o + _dot(vt_sc[pl.ds(v_off, DH), ks], p.astype(_BF16))
                return o, l + _fold8(p, jnp.sum)

            o, l = jax.lax.fori_loop(
                0, NC, pass2,
                (jnp.zeros((DH, BQ), _F32), jnp.zeros((8, BQ), _F32)))
            ot_sc[pl.ds(v_off, DH), :] = o / jnp.sum(l, axis=0, keepdims=True)
            return carry

        jax.lax.fori_loop(0, H, head, 0)

    for i in range(2, 6):
        w_copy(i).wait()

    c = D // 4
    gw = gw_ref[...].astype(_F32)

    def mix_part(mb, do_next, do_cur):
        if do_cur:
            r0 = pl.multiple_of(mb * MB, MB)
            hpre = _dot(xn_sc[pl.ds(r0, MB), :], w3_v[...])
        if do_next:
            r1 = pl.multiple_of((mb + 1) * MB, MB)
            hw = h_sc[pl.ds(r1, MB + 2 * PAD), :]
            g0 = hw[PAD - 1:PAD - 1 + MB, 0 * c:1 * c]
            g1 = hw[PAD + 1:PAD + 1 + MB, 1 * c:2 * c]
            g2 = hw[PAD - 2:PAD - 2 + MB, 2 * c:3 * c]
            g3 = hw[PAD + 2:PAD + 2 + MB, 3 * c:4 * c]
            hsft = jnp.concatenate([g0, g1, g2, g3], axis=-1).astype(_BF16)
            x1n = x_v[pl.ds(r1, MB), :].astype(_F32) + _dot(hsft, w2_v[...])
        if do_cur:
            h2 = _gelu(hpre).astype(_BF16)
            a = _dot(ot_sc[:, pl.ds(r0, MB)].T.astype(_BF16), wo_v[...])
        if do_next:
            x1_sc[pl.ds(r1, MB), :] = x1n
            xn_sc[pl.ds(r1, MB), :] = _ln(x1n).astype(_BF16)
        if do_cur:
            slot = mb % 2
            b = x1_sc[pl.ds(r0, MB), :] + _dot(h2, w4_v[...])
            xa = x_v[pl.ds(r0, MB), :].astype(_F32)
            gate = jax.nn.sigmoid(jnp.sum(xa * gw, axis=-1, keepdims=True))
            res = (gate * a + (1.0 - gate) * b).astype(o_buf.dtype)

            @pl.when(mb >= 2)
            def _():
                o_copy(mb - 2, slot).wait()

            o_buf[slot] = res
            o_copy(mb, slot).start()

    mix_part(-1, True, False)

    def mix_body(mb, carry):
        mix_part(mb, True, True)
        return carry

    jax.lax.fori_loop(0, NMB - 1, mix_body, 0)
    mix_part(NMB - 1, False, True)
    o_copy(NMB - 2, NMB % 2).wait()
    o_copy(NMB - 1, (NMB - 1) % 2).wait()


@jax.jit
def pallas_gated_mix__mha_block__mixer_s_mlp__prompt_kernel(
    A_x: jax.Array,
    A_wqkv: jax.Array,
    A_wo: jax.Array,
    B_x: jax.Array,
    B_w1: jax.Array,
    B_w2: jax.Array,
    B_w3: jax.Array,
    B_w4: jax.Array,
    gate_w: jax.Array,
):
    del B_x
    xa = A_x.reshape(S, D)
    gw = gate_w.reshape(1, D)
    hbm = pl.BlockSpec(memory_space=pl.ANY)
    kvp = max(KV, 8)

    out = pl.pallas_call(
        _kernel,
        in_specs=[hbm] * 7 + [pl.BlockSpec(memory_space=pltpu.VMEM)],
        out_specs=hbm,
        out_shape=jax.ShapeDtypeStruct((S, D), _BF16),
        scratch_shapes=[
            pltpu.VMEM((S, D), _BF16),
            pltpu.VMEM((D, 3 * D), _BF16),
            pltpu.VMEM((D, D), _BF16),
            pltpu.VMEM((D, D), _BF16),
            pltpu.VMEM((D, D), _BF16),
            pltpu.VMEM((D, F), _BF16),
            pltpu.VMEM((F, D), _BF16),
            pltpu.SemaphoreType.DMA((NPRO + 6,)),
            pltpu.SemaphoreType.DMA((2,)),
            pltpu.VMEM((2, MB, D), _BF16),
            pltpu.VMEM((NG, S, 128), _BF16),
            pltpu.VMEM((D, S), _BF16),
            pltpu.VMEM((D, S), _BF16),
            pltpu.VMEM((S + 2 * PAD, D), _F32),
            pltpu.VMEM((D, BQ), _F32),
            pltpu.VMEM((2, D, D), _BF16),
            pltpu.VMEM((S, BQ), _F32),
            pltpu.VMEM((S, BQ), _BF16),
            pltpu.VMEM((8, BQ), _F32),
            pltpu.VMEM((H, kvp, 128), _F32),
            pltpu.VMEM((DH, kvp, 128), _F32),
            pltpu.VMEM((DH, 8, BQ), _F32),
            pltpu.VMEM((2, H, PRO), _F32),
            pltpu.VMEM((S, D), _F32),
            pltpu.VMEM((S, D), _BF16),
            pltpu.SMEM((1,), jnp.int32),
        ],
        compiler_params=pltpu.CompilerParams(
            vmem_limit_bytes=110 * 1024 * 1024,
        ),
    )(xa, A_wqkv, A_wo, B_w1, B_w2, B_w3, B_w4, gw)
    return out.reshape(1, S, D)
```

```python
import math

import jax
import jax.numpy as jnp
import jax.experimental.pallas as pl
import jax.experimental.pallas.tpu as pltpu

S = 2048
D = 512
H = 32
DH = 16
F = 1792
HG = 8
NG = H // HG
KC = 128
NC = S // KC
QW = 512
NQ = S // QW
PAD = 8
PRO = 256
NPRO = S // PRO
MB = 256
NMB = S // MB
EPS = 1e-5
QSCALE = (DH ** -0.5) * math.log2(math.e)

SCORE_BOUND = 60.0
NORM2_MAX = 2.0 ** 40
V_MAX = 2.0 ** 50
V_MIN = 2.0 ** -24

_F32 = jnp.float32
_BF16 = jnp.bfloat16


def _dot(a, b):
    return jnp.dot(a, b, preferred_element_type=_F32)


def _dot_nt(a, b):
    return jax.lax.dot_general(a, b, (((1,), (1,)), ((), ())),
                               preferred_element_type=_F32)


def _ln(x):
    m = jnp.mean(x, axis=-1, keepdims=True)
    xc = x - m
    v = jnp.mean(xc * xc, axis=-1, keepdims=True)
    return xc / jnp.sqrt(v + EPS)


def _gelu(x):
    c = math.sqrt(2.0 / math.pi)
    return 0.5 * x * (1.0 + jnp.tanh(c * (x + 0.044715 * (x * x * x))))


def _fold8(x, op):
    return op(x.reshape(x.shape[0] // 8, 8, x.shape[1]), axis=0)


def _kernel(x_hbm, wqkv_hbm, wo_hbm, w1_hbm, w2_hbm, w3_hbm, w4_hbm,
            gw_ref, o_hbm,
            x_v, wqkv_v, wo_v, w1_v, w2_v, w3_v, w4_v, sems, osems, o_buf,
            k_sc, vt_sc, qt_sc, h_sc, ot_sc, wt_sc, sa, pa, la,
            g_sc, x1_sc, xn_sc, flag):

    def x_copy(c):
        return pltpu.make_async_copy(x_hbm.at[pl.ds(c * PRO, PRO), :],
                                     x_v.at[pl.ds(c * PRO, PRO), :],
                                     sems.at[c])

    def w_copy(i):
        src, dst = [(wqkv_hbm, wqkv_v), (w1_hbm, w1_v), (wo_hbm, wo_v),
                    (w2_hbm, w2_v), (w3_hbm, w3_v), (w4_hbm, w4_v)][i]
        return pltpu.make_async_copy(src, dst, sems.at[NPRO + i])

    def o_copy(mb, slot):
        return pltpu.make_async_copy(o_buf.at[slot],
                                     o_hbm.at[pl.ds(mb * MB, MB), :],
                                     osems.at[slot])

    w_copy(1).start()
    x_copy(0).start()
    x_copy(1).start()
    w_copy(0).start()
    for c in range(2, NPRO):
        x_copy(c).start()
    h_sc[0:PAD, :] = jnp.zeros((PAD, D), _F32)
    h_sc[PAD + S:PAD + S + PAD, :] = jnp.zeros((PAD, D), _F32)
    g_sc[0] = jnp.zeros((H, PRO), _F32)
    g_sc[1] = jnp.zeros((H, PRO), _F32)
    w_copy(1).wait()

    grp = (jax.lax.broadcasted_iota(jnp.int32, (H, D), 1) // DH ==
           jax.lax.broadcasted_iota(jnp.int32, (H, D), 0)
           ).astype(_F32).astype(_BF16)

    def pro_part(c, vmax, do_h, do_qkv, pre=None):
        if do_h:
            r1 = pl.multiple_of((c + 2) * PRO, PRO)
            x_copy(c + 2).wait()
        if do_qkv:
            r0 = pl.multiple_of(c * PRO, PRO)
            x = x_v[pl.ds(r0, PRO), :]
            k = _dot(x, wqkv_v[:, D:2 * D]).astype(_BF16)
            for g in range(NG):
                k_sc[g, pl.ds(r0, PRO), :] = k[:, g * 128:(g + 1) * 128]
        if pre is not None:
            pre()
        if do_h:
            xn = _ln(x_v[pl.ds(r1, PRO), :].astype(_F32)).astype(_BF16)
            hpre = _dot(xn, w1_v[...])
        if do_qkv:
            qt = (_dot_nt(wt_sc[0], x) * QSCALE).astype(_BF16)
            qt_sc[:, pl.ds(r0, PRO)] = qt
        if do_h:
            h_sc[pl.ds(PAD + r1, PRO), :] = (
                _gelu(hpre).astype(_BF16).astype(_F32))
        if do_qkv:
            vt = _dot_nt(wt_sc[1], x).astype(_BF16)
            vt_sc[:, pl.ds(r0, PRO)] = vt
            k32 = k.astype(_F32)
            q32 = qt.astype(_F32)
            g_sc[0] = jnp.maximum(g_sc[0],
                                  _dot(grp, (q32 * q32).astype(_BF16)))
            g_sc[1] = jnp.maximum(g_sc[1],
                                  _dot_nt(grp, (k32 * k32).astype(_BF16)))
            vmax = jnp.maximum(vmax,
                               _fold8(jnp.abs(vt.astype(_F32)).T, jnp.max))
        return vmax

    def transpose_weights():
        wt_sc[0] = wqkv_v[:, 0:D].astype(_F32).T.astype(_BF16)
        wt_sc[1] = wqkv_v[:, 2 * D:3 * D].astype(_F32).T.astype(_BF16)

    pro_part(-2, None, True, False)
    pro_part(-1, None, True, False)
    w_copy(0).wait()
    for i in (3, 2, 4, 5):
        w_copy(i).start()
    vmax = pro_part(0, jnp.zeros((8, D), _F32), True, True, transpose_weights)
    vmax = jax.lax.fori_loop(
        1, NPRO - 2, lambda c, vm: pro_part(c, vm, True, True), vmax)
    vmax = jax.lax.fori_loop(
        NPRO - 2, NPRO, lambda c, vm: pro_part(c, vm, False, True), vmax)

    vcol = jnp.max(vmax, axis=0, keepdims=True)
    q2 = jnp.max(g_sc[0], axis=1, keepdims=True)
    k2 = jnp.max(g_sc[1], axis=1, keepdims=True)
    ok_s = ((q2 * k2 * 1.03 <= SCORE_BOUND * SCORE_BOUND) &
            (q2 <= NORM2_MAX) & (k2 <= NORM2_MAX)).astype(_F32)
    ok_v = ((vcol <= V_MAX) & ((vcol >= V_MIN) | (vcol == 0.0))).astype(_F32)
    ok = jnp.minimum(jnp.min(ok_s), jnp.min(ok_v))
    flag[0] = (ok > 0.5).astype(jnp.int32)

    rows = jax.lax.broadcasted_iota(jnp.int32, (128, S), 0)

    def make_qm(h):
        g = h // HG
        hl = h % HG
        qg = qt_sc[pl.ds(pl.multiple_of(g * 128, 128), 128), :]
        return g, jnp.where((rows >> 4) == hl, qg, jnp.zeros_like(qg))

    def fstage(h, do_pv, do_qk):
        o = [None] * NQ
        l_new = [None] * NQ
        if do_pv:
            l_old = jnp.sum(la[...], axis=0, keepdims=True)
            v_off = pl.multiple_of(h * DH, DH)
        if do_qk:
            g, qm = make_qm(h + 1)
        for c in range(NC):
            ks = slice(c * KC, (c + 1) * KC)
            for j in range(NQ):
                qs = slice(j * QW, (j + 1) * QW)
                if do_pv:
                    oc = _dot(vt_sc[pl.ds(v_off, DH), ks], pa[ks, qs])
                    o[j] = oc if o[j] is None else o[j] + oc
                if do_qk:
                    p = jnp.exp2(_dot(k_sc[g, ks, :], qm[:, qs]))
                    pa[ks, qs] = p.astype(_BF16)
                    lc = _fold8(p, jnp.sum)
                    l_new[j] = lc if l_new[j] is None else l_new[j] + lc
        if do_pv:
            ot_sc[pl.ds(v_off, DH), :] = jnp.concatenate(o, axis=1) / l_old
        if do_qk:
            la[...] = jnp.concatenate(l_new, axis=1)

    @pl.when(flag[0] == 1)
    def _fast():
        fstage(-1, False, True)

        def body(h, carry):
            fstage(h, True, True)
            return carry

        jax.lax.fori_loop(0, H - 1, body, 0)

    @pl.when(flag[0] != 1)
    def _general():
        def head(h, last):
            g, qm = make_qm(h)
            v_off = pl.multiple_of(h * DH, DH)

            def pass1(c, m):
                ks = pl.ds(pl.multiple_of(c * KC, KC), KC)
                s = _dot(k_sc[g, ks, :], qm)
                sa[ks, :] = s
                return jnp.maximum(m, _fold8(s, jnp.max))

            m8 = jax.lax.fori_loop(
                0, NC, pass1, jnp.full((8, S), -jnp.inf, _F32))
            m = jnp.max(m8, axis=0, keepdims=True)

            def pass2(c, carry2):
                o, l = carry2
                ks = pl.ds(pl.multiple_of(c * KC, KC), KC)
                p = jnp.exp2(sa[ks, :] - m)
                pb = p.astype(_BF16)
                if last:
                    pa[ks, :] = pb
                else:
                    o = o + _dot(vt_sc[pl.ds(v_off, DH), ks], pb)
                return o, l + _fold8(p, jnp.sum)

            o, l = jax.lax.fori_loop(
                0, NC, pass2,
                (jnp.zeros((DH, S), _F32), jnp.zeros((8, S), _F32)))
            if last:
                la[...] = l
            else:
                ot_sc[pl.ds(v_off, DH), :] = (
                    o / jnp.sum(l, axis=0, keepdims=True))

        def body(h, carry):
            head(h, False)
            return carry

        jax.lax.fori_loop(0, H - 1, body, 0)
        head(H - 1, True)

    for i in range(2, 6):
        w_copy(i).wait()

    c = D // 4
    gw = gw_ref[...].astype(_F32)

    def mix_part(mb, do_next, do_cur):
        if do_cur:
            r0 = pl.multiple_of(mb * MB, MB)
            hpre = _dot(xn_sc[pl.ds(r0, MB), :], w3_v[...])
        if do_next:
            r1 = pl.multiple_of((mb + 1) * MB, MB)
            hw = h_sc[pl.ds(r1, MB + 2 * PAD), :]
            g0 = hw[PAD - 1:PAD - 1 + MB, 0 * c:1 * c]
            g1 = hw[PAD + 1:PAD + 1 + MB, 1 * c:2 * c]
            g2 = hw[PAD - 2:PAD - 2 + MB, 2 * c:3 * c]
            g3 = hw[PAD + 2:PAD + 2 + MB, 3 * c:4 * c]
            hsft = jnp.concatenate([g0, g1, g2, g3], axis=-1).astype(_BF16)
            x1n = x_v[pl.ds(r1, MB), :].astype(_F32) + _dot(hsft, w2_v[...])
        if do_cur:
            h2 = _gelu(hpre).astype(_BF16)
            a = _dot(ot_sc[:, pl.ds(r0, MB)].T.astype(_BF16), wo_v[...])
        if do_next:
            x1_sc[pl.ds(r1, MB), :] = x1n
            xn_sc[pl.ds(r1, MB), :] = _ln(x1n).astype(_BF16)
        if do_cur:
            slot = mb % 2
            b = x1_sc[pl.ds(r0, MB), :] + _dot(h2, w4_v[...])
            xa = x_v[pl.ds(r0, MB), :].astype(_F32)
            gate = jax.nn.sigmoid(jnp.sum(xa * gw, axis=-1, keepdims=True))
            res = (gate * a + (1.0 - gate) * b).astype(o_buf.dtype)

            @pl.when(mb >= 2)
            def _():
                o_copy(mb - 2, slot).wait()

            o_buf[slot] = res
            o_copy(mb, slot).start()

    mix_part(-1, True, False)
    fstage(H - 1, True, False)

    def mix_body(mb, carry):
        mix_part(mb, True, True)
        return carry

    jax.lax.fori_loop(0, NMB - 1, mix_body, 0)
    mix_part(NMB - 1, False, True)
    o_copy(NMB - 2, NMB % 2).wait()
    o_copy(NMB - 1, (NMB - 1) % 2).wait()


@jax.jit
def pallas_gated_mix__mha_block__mixer_s_mlp__prompt_kernel(
    A_x: jax.Array,
    A_wqkv: jax.Array,
    A_wo: jax.Array,
    B_x: jax.Array,
    B_w1: jax.Array,
    B_w2: jax.Array,
    B_w3: jax.Array,
    B_w4: jax.Array,
    gate_w: jax.Array,
):
    del B_x
    xa = A_x.reshape(S, D)
    gw = gate_w.reshape(1, D)
    hbm = pl.BlockSpec(memory_space=pl.ANY)

    out = pl.pallas_call(
        _kernel,
        in_specs=[hbm] * 7 + [pl.BlockSpec(memory_space=pltpu.VMEM)],
        out_specs=hbm,
        out_shape=jax.ShapeDtypeStruct((S, D), _BF16),
        scratch_shapes=[
            pltpu.VMEM((S, D), _BF16),
            pltpu.VMEM((D, 3 * D), _BF16),
            pltpu.VMEM((D, D), _BF16),
            pltpu.VMEM((D, D), _BF16),
            pltpu.VMEM((D, D), _BF16),
            pltpu.VMEM((D, F), _BF16),
            pltpu.VMEM((F, D), _BF16),
            pltpu.SemaphoreType.DMA((NPRO + 6,)),
            pltpu.SemaphoreType.DMA((2,)),
            pltpu.VMEM((2, MB, D), _BF16),
            pltpu.VMEM((NG, S, 128), _BF16),
            pltpu.VMEM((D, S), _BF16),
            pltpu.VMEM((D, S), _BF16),
            pltpu.VMEM((S + 2 * PAD, D), _F32),
            pltpu.VMEM((D, S), _F32),
            pltpu.VMEM((2, D, D), _BF16),
            pltpu.VMEM((S, S), _F32),
            pltpu.VMEM((S, S), _BF16),
            pltpu.VMEM((8, S), _F32),
            pltpu.VMEM((2, H, PRO), _F32),
            pltpu.VMEM((S, D), _F32),
            pltpu.VMEM((S, D), _BF16),
            pltpu.SMEM((1,), jnp.int32),
        ],
        compiler_params=pltpu.CompilerParams(
            vmem_limit_bytes=110 * 1024 * 1024,
        ),
    )(xa, A_wqkv, A_wo, B_w1, B_w2, B_w3, B_w4, gw)
    return out.reshape(1, S, D)
```

```python
import math

import jax
import jax.numpy as jnp
import jax.experimental.pallas as pl
import jax.experimental.pallas.tpu as pltpu

S = 2048
D = 512
H = 32
DH = 16
F = 1792
HG = 8
NG = H // HG
KC = 128
NC = S // KC
QW = 512
NQ = S // QW
PAD = 8
PRO = 256
NPRO = S // PRO
MB = 256
NMB = S // MB
EPS = 1e-5
KV = 96
KV0 = S - KV
PK = 8
V_END = 60
QSCALE = (DH ** -0.5) * math.log2(math.e)

SCORE_BOUND = 60.0
NORM2_MAX = 2.0 ** 40
V_MAX = 2.0 ** 50
V_MIN = 2.0 ** -24

_F32 = jnp.float32
_BF16 = jnp.bfloat16


def _dot(a, b):
    return jnp.dot(a, b, preferred_element_type=_F32)


def _dot_nt(a, b):
    return jax.lax.dot_general(a, b, (((1,), (1,)), ((), ())),
                               preferred_element_type=_F32)


def _ln(x):
    m = jnp.mean(x, axis=-1, keepdims=True)
    xc = x - m
    v = jnp.mean(xc * xc, axis=-1, keepdims=True)
    return xc / jnp.sqrt(v + EPS)


def _gelu(x):
    c = math.sqrt(2.0 / math.pi)
    return 0.5 * x * (1.0 + jnp.tanh(c * (x + 0.044715 * (x * x * x))))


def _fold8(x, op):
    return op(x.reshape(x.shape[0] // 8, 8, x.shape[1]), axis=0)


def _kernel(x_hbm, wqkv_hbm, wo_hbm, w1_hbm, w2_hbm, w3_hbm, w4_hbm,
            gw_ref, o_hbm,
            x_v, wqkv_v, wo_v, w1_v, w2_v, w3_v, w4_v, sems, osems, o_buf,
            k_sc, vt_sc, qt_sc, h_sc, ot_sc, wt_sc, sa, pa, la,
            g_sc, x1_sc, xn_sc, kv_sc, qb, flag):

    def x_copy(c):
        return pltpu.make_async_copy(x_hbm.at[pl.ds(c * PRO, PRO), :],
                                     x_v.at[pl.ds(c * PRO, PRO), :],
                                     sems.at[c])

    def w_copy(i):
        src, dst = [(wqkv_hbm, wqkv_v), (w1_hbm, w1_v), (wo_hbm, wo_v),
                    (w2_hbm, w2_v), (w3_hbm, w3_v), (w4_hbm, w4_v)][i]
        return pltpu.make_async_copy(src, dst, sems.at[NPRO + i])

    def o_copy(mb, slot):
        return pltpu.make_async_copy(o_buf.at[slot],
                                     o_hbm.at[pl.ds(mb * MB, MB), :],
                                     osems.at[slot])

    w_copy(1).start()
    x_copy(0).start()
    x_copy(1).start()
    w_copy(0).start()
    for c in range(2, NPRO):
        x_copy(c).start()
    h_sc[0:PAD, :] = jnp.zeros((PAD, D), _F32)
    h_sc[PAD + S:PAD + S + PAD, :] = jnp.zeros((PAD, D), _F32)
    g_sc[0] = jnp.zeros((H, PRO), _F32)
    g_sc[1] = jnp.zeros((H, PRO), _F32)
    w_copy(1).wait()

    grp = (jax.lax.broadcasted_iota(jnp.int32, (H, D), 1) // DH ==
           jax.lax.broadcasted_iota(jnp.int32, (H, D), 0)
           ).astype(_F32).astype(_BF16)

    def pro_part(c, vmax, do_h, do_qkv, pre=None):
        if do_h:
            r1 = pl.multiple_of((c + 2) * PRO, PRO)
            x_copy(c + 2).wait()
        if do_qkv:
            r0 = pl.multiple_of(c * PRO, PRO)
            x = x_v[pl.ds(r0, PRO), :]
            k = _dot(x, wqkv_v[:, D:2 * D]).astype(_BF16)
            for g in range(NG):
                k_sc[g, pl.ds(r0, PRO), :] = k[:, g * 128:(g + 1) * 128]
        if pre is not None:
            pre()
        if do_h:
            xn = _ln(x_v[pl.ds(r1, PRO), :].astype(_F32)).astype(_BF16)
            hpre = _dot(xn, w1_v[...])
        if do_qkv:
            qt = (_dot_nt(wt_sc[0], x) * QSCALE).astype(_BF16)
            qt_sc[:, pl.ds(r0, PRO)] = qt
        if do_h:
            h_sc[pl.ds(PAD + r1, PRO), :] = (
                _gelu(hpre).astype(_BF16).astype(_F32))
        if do_qkv:
            vt = _dot_nt(wt_sc[1], x).astype(_BF16)
            vt_sc[:, pl.ds(r0, PRO)] = vt
            k32 = k.astype(_F32)
            q32 = qt.astype(_F32)
            g_sc[0] = jnp.maximum(g_sc[0],
                                  _dot(grp, (q32 * q32).astype(_BF16)))
            g_sc[1] = jnp.maximum(g_sc[1],
                                  _dot_nt(grp, (k32 * k32).astype(_BF16)))
            vmax = jnp.maximum(vmax,
                               _fold8(jnp.abs(vt.astype(_F32)).T, jnp.max))
        return vmax

    def transpose_weights():
        wt_sc[0] = wqkv_v[:, 0:D].astype(_F32).T.astype(_BF16)
        wt_sc[1] = wqkv_v[:, 2 * D:3 * D].astype(_F32).T.astype(_BF16)

    pro_part(-2, None, True, False)
    pro_part(-1, None, True, False)
    w_copy(0).wait()
    for i in (3, 2, 4, 5):
        w_copy(i).start()
    vmax = pro_part(0, jnp.zeros((8, D), _F32), True, True, transpose_weights)
    vmax = jax.lax.fori_loop(
        1, NPRO - 2, lambda c, vm: pro_part(c, vm, True, True), vmax)
    vmax = jax.lax.fori_loop(
        NPRO - 2, NPRO, lambda c, vm: pro_part(c, vm, False, True), vmax)

    vcol = jnp.max(vmax, axis=0, keepdims=True)
    q2 = jnp.max(g_sc[0], axis=1, keepdims=True)
    k2 = jnp.max(g_sc[1], axis=1, keepdims=True)
    ok_s = ((q2 * k2 * 1.03 <= SCORE_BOUND * SCORE_BOUND) &
            (q2 <= NORM2_MAX) & (k2 <= NORM2_MAX)).astype(_F32)
    ok_v = ((vcol <= V_MAX) & ((vcol >= V_MIN) | (vcol == 0.0))).astype(_F32)
    ok = jnp.minimum(jnp.min(ok_s), jnp.min(ok_v))
    flag[0] = (ok > 0.5).astype(jnp.int32)

    rows = jax.lax.broadcasted_iota(jnp.int32, (128, S), 0)

    def make_qm(h):
        g = h // HG
        hl = h % HG
        qg = qt_sc[pl.ds(pl.multiple_of(g * 128, 128), 128), :]
        return g, jnp.where((rows >> 4) == hl, qg, jnp.zeros_like(qg))

    def prep_q(h):
        h = jnp.minimum(h, H - 1)
        q = qt_sc[pl.ds(pl.multiple_of(h * DH, DH), DH), :].astype(_F32)
        for d in range(DH):
            qb[d] = jnp.broadcast_to(q[d:d + 1, :], (8, S))

    def vpu_piece(h, i, j, dep):
        r0 = i * PK
        k = kv_sc[h, r0:r0 + PK, :]
        if dep is not None:
            k = k + jnp.minimum(dep[0:PK, 0:128], 0.0)
        accs = [None] * (QW // 128)
        for d in range(DH):
            kk = jnp.broadcast_to(k[:, d:d + 1], (PK, 128))
            for n in range(QW // 128):
                ns = slice(j * QW + n * 128, j * QW + (n + 1) * 128)
                tt = kk * qb[d, :, ns]
                accs[n] = tt if accs[n] is None else accs[n] + tt
        p = jnp.exp2(jnp.concatenate(accs, axis=1))
        pa[KV0 + r0:KV0 + r0 + PK, j * QW:(j + 1) * QW] = p.astype(_BF16)
        return p

    order = [NC - 1] + list(range(NC - 1))

    def fstage(h, do_pv, do_qk):
        o = [None] * NQ
        l_new = [None] * NQ
        vp = []
        if do_pv:
            l_old = jnp.sum(la[...], axis=0, keepdims=True)
            v_off = pl.multiple_of(h * DH, DH)
        if do_qk:
            g, qm = make_qm(h + 1)
            vp = sorted((j, i) for i in range(KV // PK) for j in range(NQ))
        n_vp = len(vp)
        slot = 0
        for c in order:
            ks = slice(c * KC, (c + 1) * KC)
            lo, hi = c * KC, min((c + 1) * KC, KV0)
            for j in range(NQ):
                qs = slice(j * QW, (j + 1) * QW)
                if do_pv:
                    oc = _dot(vt_sc[pl.ds(v_off, DH), ks], pa[ks, qs])
                    o[j] = oc if o[j] is None else o[j] + oc
                if do_qk:
                    p = jnp.exp2(_dot(k_sc[g, lo:hi, :], qm[:, qs]))
                    pa[lo:hi, qs] = p.astype(_BF16)
                    lc = _fold8(p, jnp.sum)
                    l_new[j] = lc if l_new[j] is None else l_new[j] + lc
                while (vp and vp[0][0] <= slot and
                       (n_vp - len(vp)) * (V_END + 1) < (slot + 1) * n_vp):
                    jj, i = vp.pop(0)
                    l_new[jj] = l_new[jj] + vpu_piece(h + 1, i, jj, p)
                slot += 1
        assert not vp
        if do_pv:
            ot_sc[pl.ds(v_off, DH), :] = jnp.concatenate(o, axis=1) / l_old
        if do_qk:
            la[...] = jnp.concatenate(l_new, axis=1)
            prep_q(h + 2)

    @pl.when(flag[0] == 1)
    def _prep():
        for g in range(NG):
            kg = k_sc[g, KV0:S, :].astype(_F32)
            for hl in range(HG):
                kv_sc[g * HG + hl] = (
                    kg if hl == 0 else pltpu.roll(kg, 128 - hl * DH, 1))
        prep_q(0)

    @pl.when(flag[0] == 1)
    def _fast():
        fstage(-1, False, True)

        def body(h, carry):
            fstage(h, True, True)
            return carry

        jax.lax.fori_loop(0, H - 1, body, 0)

    @pl.when(flag[0] != 1)
    def _general():
        def head(h, last):
            g, qm = make_qm(h)
            v_off = pl.multiple_of(h * DH, DH)

            def pass1(c, m):
                ks = pl.ds(pl.multiple_of(c * KC, KC), KC)
                s = _dot(k_sc[g, ks, :], qm)
                sa[ks, :] = s
                return jnp.maximum(m, _fold8(s, jnp.max))

            m8 = jax.lax.fori_loop(
                0, NC, pass1, jnp.full((8, S), -jnp.inf, _F32))
            m = jnp.max(m8, axis=0, keepdims=True)

            def pass2(c, carry2):
                o, l = carry2
                ks = pl.ds(pl.multiple_of(c * KC, KC), KC)
                p = jnp.exp2(sa[ks, :] - m)
                pb = p.astype(_BF16)
                if last:
                    pa[ks, :] = pb
                else:
                    o = o + _dot(vt_sc[pl.ds(v_off, DH), ks], pb)
                return o, l + _fold8(p, jnp.sum)

            o, l = jax.lax.fori_loop(
                0, NC, pass2,
                (jnp.zeros((DH, S), _F32), jnp.zeros((8, S), _F32)))
            if last:
                la[...] = l
            else:
                ot_sc[pl.ds(v_off, DH), :] = (
                    o / jnp.sum(l, axis=0, keepdims=True))

        def body(h, carry):
            head(h, False)
            return carry

        jax.lax.fori_loop(0, H - 1, body, 0)
        head(H - 1, True)

    for i in range(2, 6):
        w_copy(i).wait()

    c = D // 4
    gw = gw_ref[...].astype(_F32)

    def mix_part(mb, do_next, do_cur):
        if do_cur:
            r0 = pl.multiple_of(mb * MB, MB)
            hpre = _dot(xn_sc[pl.ds(r0, MB), :], w3_v[...])
        if do_next:
            r1 = pl.multiple_of((mb + 1) * MB, MB)
            hw = h_sc[pl.ds(r1, MB + 2 * PAD), :]
            g0 = hw[PAD - 1:PAD - 1 + MB, 0 * c:1 * c]
            g1 = hw[PAD + 1:PAD + 1 + MB, 1 * c:2 * c]
            g2 = hw[PAD - 2:PAD - 2 + MB, 2 * c:3 * c]
            g3 = hw[PAD + 2:PAD + 2 + MB, 3 * c:4 * c]
            hsft = jnp.concatenate([g0, g1, g2, g3], axis=-1).astype(_BF16)
            x1n = x_v[pl.ds(r1, MB), :].astype(_F32) + _dot(hsft, w2_v[...])
        if do_cur:
            h2 = _gelu(hpre).astype(_BF16)
            a = _dot(ot_sc[:, pl.ds(r0, MB)].T.astype(_BF16), wo_v[...])
        if do_next:
            x1_sc[pl.ds(r1, MB), :] = x1n
            xn_sc[pl.ds(r1, MB), :] = _ln(x1n).astype(_BF16)
        if do_cur:
            slot = mb % 2
            b = x1_sc[pl.ds(r0, MB), :] + _dot(h2, w4_v[...])
            xa = x_v[pl.ds(r0, MB), :].astype(_F32)
            gate = jax.nn.sigmoid(jnp.sum(xa * gw, axis=-1, keepdims=True))
            res = (gate * a + (1.0 - gate) * b).astype(o_buf.dtype)

            @pl.when(mb >= 2)
            def _():
                o_copy(mb - 2, slot).wait()

            o_buf[slot] = res
            o_copy(mb, slot).start()

    mix_part(-1, True, False)
    fstage(H - 1, True, False)

    def mix_body(mb, carry):
        mix_part(mb, True, True)
        return carry

    jax.lax.fori_loop(0, NMB - 1, mix_body, 0)
    mix_part(NMB - 1, False, True)
    o_copy(NMB - 2, NMB % 2).wait()
    o_copy(NMB - 1, (NMB - 1) % 2).wait()


@jax.jit
def pallas_gated_mix__mha_block__mixer_s_mlp__prompt_kernel(
    A_x: jax.Array,
    A_wqkv: jax.Array,
    A_wo: jax.Array,
    B_x: jax.Array,
    B_w1: jax.Array,
    B_w2: jax.Array,
    B_w3: jax.Array,
    B_w4: jax.Array,
    gate_w: jax.Array,
):
    del B_x
    xa = A_x.reshape(S, D)
    gw = gate_w.reshape(1, D)
    hbm = pl.BlockSpec(memory_space=pl.ANY)

    out = pl.pallas_call(
        _kernel,
        in_specs=[hbm] * 7 + [pl.BlockSpec(memory_space=pltpu.VMEM)],
        out_specs=hbm,
        out_shape=jax.ShapeDtypeStruct((S, D), _BF16),
        scratch_shapes=[
            pltpu.VMEM((S, D), _BF16),
            pltpu.VMEM((D, 3 * D), _BF16),
            pltpu.VMEM((D, D), _BF16),
            pltpu.VMEM((D, D), _BF16),
            pltpu.VMEM((D, D), _BF16),
            pltpu.VMEM((D, F), _BF16),
            pltpu.VMEM((F, D), _BF16),
            pltpu.SemaphoreType.DMA((NPRO + 6,)),
            pltpu.SemaphoreType.DMA((2,)),
            pltpu.VMEM((2, MB, D), _BF16),
            pltpu.VMEM((NG, S, 128), _BF16),
            pltpu.VMEM((D, S), _BF16),
            pltpu.VMEM((D, S), _BF16),
            pltpu.VMEM((S + 2 * PAD, D), _F32),
            pltpu.VMEM((D, S), _F32),
            pltpu.VMEM((2, D, D), _BF16),
            pltpu.VMEM((S, S), _F32),
            pltpu.VMEM((S, S), _BF16),
            pltpu.VMEM((8, S), _F32),
            pltpu.VMEM((2, H, PRO), _F32),
            pltpu.VMEM((S, D), _F32),
            pltpu.VMEM((S, D), _BF16),
            pltpu.VMEM((H, KV, 128), _F32),
            pltpu.VMEM((DH, 8, S), _F32),
            pltpu.SMEM((1,), jnp.int32),
        ],
        compiler_params=pltpu.CompilerParams(
            vmem_limit_bytes=110 * 1024 * 1024,
        ),
    )(xa, A_wqkv, A_wo, B_w1, B_w2, B_w3, B_w4, gw)
    return out.reshape(1, S, D)
```
